```python
import os as _os
_os.environ.setdefault('JAX_PLATFORMS', 'cpu')
import jax
import jax.numpy as jnp

def _softmax(x, axis=-1):
    return jax.nn.softmax(x, axis=axis)

def _gelu(x):
    return jax.nn.gelu(x, approximate=True)

def _silu(x):
    return jax.nn.silu(x)

def _sigmoid(x):
    return jax.nn.sigmoid(x)

def _layernorm(x, axis=-1, eps=1e-05):
    m = jnp.mean(x, axis=axis, keepdims=True)
    v = jnp.var(x, axis=axis, keepdims=True)
    return (x - m) / jnp.sqrt(v + eps)

def _scatter_add(tgt, idx, src, axis=0):
    return tgt.at[idx].add(src)

def _segment_sum(src, seg, n):
    return jax.ops.segment_sum(src, seg, n)

class _Rng:

    def __init__(self, key):
        self._k = key

    def _next(self):
        self._k, sub = jax.random.split(self._k)
        return sub

    def normal(self, shape):
        return jax.random.normal(self._next(), shape, dtype=jnp.bfloat16)

    def randint(self, lo, hi, shape):
        return jax.random.randint(self._next(), shape, lo, hi, dtype=jnp.int32)

    def uniform(self, shape, lo=0.0, hi=1.0):
        return jax.random.uniform(self._next(), shape, jnp.bfloat16, lo, hi)

    def permutation(self, n):
        return jax.random.permutation(self._next(), n)
kernel_name = 'sequential_preLN__linear_attn_block__mixer_gmlp__prompt'

def setup_inputs():
    _rng = _Rng(jax.random.key(int.from_bytes(__import__("os").urandom(4), "little")))
    _w = lambda a: (lambda t: t.astype(jnp.bfloat16) if jnp.issubdtype(t.dtype, jnp.floating) else t)(jnp.asarray(a))

    def _A_setup():
        B, S, D = (1, 2048, 512)
        return {'x': _w((lambda *s: _rng.normal(s) * 0.05)(B, S, D)), 'wqkv': _w((lambda *s: _rng.normal(s) * 0.05)(D, 3 * D)), 'wo': _w((lambda *s: _rng.normal(s) * 0.05)(D, D))}
    _A_in = _A_setup()

    def _B_setup():
        B, S, D, F = (1, 2048, 512, 1792)
        Fh = F // 2
        return {'x': _w((lambda *s: _rng.normal(s) * 0.05)(B, S, D)), 'w_in': _w((lambda *s: _rng.normal(s) * 0.4)(D, 2 * Fh)), 'w_sp': _w(0.01 * (lambda *s: _rng.normal(s) * 0.4)(S, S)), 'b_sp': _w(1.0 + 0.01 * (lambda *s: _rng.normal(s) * 0.05)(S)), 'w_out': _w((lambda *s: _rng.normal(s) * 0.05)(Fh, D))}
    _B_in = _B_setup()
    return {'A_x': _A_in['x'], 'A_wqkv': _A_in['wqkv'], 'A_wo': _A_in['wo'], 'B_x': _B_in['x'], 'B_w_in': _B_in['w_in'], 'B_w_sp': _B_in['w_sp'], 'B_b_sp': _B_in['b_sp'], 'B_w_out': _B_in['w_out']}

def reference(A_x, A_wqkv, A_wo, B_x, B_w_in, B_w_sp, B_b_sp, B_w_out):

    def _A_ref(x, wqkv, wo):
        B, S, D = x.shape
        H = 32
        Dh = D // H
        qkv = (lambda x, *d: x.transpose(*d))((x @ wqkv).reshape(B, S, 3, H, Dh), 2, 0, 3, 1, 4)
        q, k, v = (qkv[0], qkv[1], qkv[2])
        phi = lambda t: jnp.where(t > 0, t + 1, jnp.exp(t)) + 1e-06
        pq, pk = (phi(q), phi(k))
        kv = jnp.einsum('bhsd,bhse->bhde', pk, v)
        z = jnp.einsum('bhsd->bhd', pk)
        num = jnp.einsum('bhqd,bhde->bhqe', pq, kv)
        den = jnp.einsum('bhqd,bhd->bhq', pq, z)[..., None] + 1e-06
        o = num / den
        return (lambda x, *d: x.transpose(*d))(o, 0, 2, 1, 3).reshape(B, S, D) @ wo

    def _B_ref(x, w_in, w_sp, b_sp, w_out):
        B, S, D = x.shape
        F = w_in.shape[-1]
        Fh = F // 2
        z = _gelu(jnp.einsum('bsd,df->bsf', x, w_in))
        z1 = z[..., :Fh].copy()
        z2 = _layernorm(z[..., Fh:], axis=-1)
        g = jnp.einsum('ts,bsf->btf', w_sp, z2) + b_sp[None, :, None]
        return jnp.einsum('bsf,fd->bsd', z1 * g, w_out)
    x = A_x
    h = x + _A_ref(_layernorm(x, axis=-1), A_wqkv, A_wo)
    h2 = h + _B_ref(_layernorm(h, axis=-1), B_w_in, B_w_sp, B_b_sp, B_w_out)
    return h2
```

```python
import jax
import jax.numpy as jnp
from jax import lax
import jax.experimental.pallas as pl
import jax.experimental.pallas.tpu as pltpu

S, D, H, DH = 2048, 512, 32, 16
F, FH = 1792, 896
TM = 256
NB = S // TM
G = 128
NG = D // G
NDEF = 3

import contextlib


def _scope(n):
    return contextlib.nullcontext()


f32 = jnp.float32
bf16 = jnp.bfloat16


def _ln(x):
    m = jnp.mean(x, axis=-1, keepdims=True)
    xc = x - m
    v = jnp.mean(xc * xc, axis=-1, keepdims=True)
    return xc * lax.rsqrt(v + 1e-5)


def _phi(t):
    return jnp.where(t > 0, t + 1.0, jnp.exp(t)) + 1e-6


def _gelu(x):
    c = 0.7978845608028654
    return 0.5 * x * (1.0 + jnp.tanh(c * (x + 0.044715 * (x * x * x))))


def _dot(a, b):
    return jnp.dot(a, b, preferred_element_type=f32)


def _dot_nt(a, b):
    return lax.dot_general(a, b, (((1,), (1,)), ((), ())), preferred_element_type=f32)


def _div(a, b):
    r = pl.reciprocal(b, approx=True)
    r = r * (2.0 - b * r)
    return a * r


def _kernel(x_hbm, wqkv_hbm, wo_hbm, win_hbm, wsp_hbm, b_hbm, wout_hbm, out_hbm,
            x_v, wqkv_v, wo_v, win_v, wsp_v, b_v, wout_v,
            wkT_v, xn_v, pkT_v, pq_v, kv_v, zs_v, m_v, zm_v, h_v, z1_v, z2_v, g_v, out_v,
            sem, sem_o):
    def rows(i):
        if isinstance(i, int):
            return pl.ds(i * TM, TM)
        return pl.ds(pl.multiple_of(i * TM, TM), TM)

    def cp_xr(lo, n, s):
        return pltpu.make_async_copy(x_hbm.at[pl.ds(lo * TM, n * TM)], x_v.at[pl.ds(lo * TM, n * TM)], sem.at[s])

    def cp_o(i):
        return pltpu.make_async_copy(out_v.at[pl.ds(i * TM, TM)], out_hbm.at[pl.ds(i * TM, TM)], sem_o.at[i])

    def cp_w3(j):
        return pltpu.make_async_copy(wqkv_hbm.at[:, pl.ds(j * D, D)], wqkv_v.at[:, pl.ds(j * D, D)], sem.at[3 + j])

    cp_x01 = cp_xr(0, 2, 0)
    cp_x2 = cp_xr(2, 1, 1)
    cp_x3 = cp_xr(3, NB - 3, 2)
    cp_wo = pltpu.make_async_copy(wo_hbm, wo_v, sem.at[6])
    cp_win = pltpu.make_async_copy(win_hbm, win_v, sem.at[7])
    cp_wout = pltpu.make_async_copy(wout_hbm, wout_v, sem.at[8])
    cp_b = pltpu.make_async_copy(b_hbm, b_v, sem.at[9])
    cp_sp = pltpu.make_async_copy(wsp_hbm, wsp_v, sem.at[10])

    cp_x01.start()
    cp_w3(0).start()
    cp_w3(1).start()
    cp_w3(2).start()
    cp_x2.start()
    cp_x3.start()

    def lnx(i):
        r = rows(i)
        xn_v[r, :] = _ln(x_v[r, :].astype(f32)).astype(bf16)

    def kproj(i):
        r = rows(i)
        pkT = _phi(_dot_nt(wkT_v[...], xn_v[r, :]))
        zpart = pkT[:, 0:128]
        for t in range(1, TM // 128):
            zpart = zpart + pkT[:, t * 128:(t + 1) * 128]
        if i == 0:
            zs_v[...] = zpart
        else:
            zs_v[...] += zpart
        pkT_v[:, r] = pkT.astype(bf16)

    def qproj(i):
        r = rows(i)
        pq_v[r, :] = _phi(_dot(xn_v[r, :], wqkv_v[:, 0:D])).astype(bf16)

    with _scope('PRO'):
        cp_x01.wait()
        lnx(0)
        lnx(1)
        cp_w3(0).wait()
        qproj(0)
        cp_w3(1).wait()
        qproj(1)
        wkT_v[...] = wqkv_v[:, D:2 * D].astype(f32).T.astype(bf16)
        kproj(0)
        cp_w3(2).wait()
        cp_x2.wait()

    def p1_body(i):
        r = rows(i)
        v = _dot(xn_v[r, :], wqkv_v[:, 2 * D:3 * D]).astype(bf16)
        if i + 2 < NB:
            lnx(i + 2)
        if i + 1 < NB:
            kproj(i + 1)
        if i + 2 < NB - NDEF:
            qproj(i + 2)
        for j in range(NG):
            kvj = _dot(pkT_v[j * G:(j + 1) * G, r], v[:, j * G:(j + 1) * G])
            if i == 0:
                kv_v[j * G:(j + 1) * G, :] = kvj
            else:
                kv_v[j * G:(j + 1) * G, :] += kvj

    with _scope('P1'):
        p1_body(0)
        cp_x3.wait()
        cp_wo.start()
        cp_win.start()
        cp_b.start()
        cp_sp.start(priority=1)
        cp_wout.start(priority=1)
        for i in range(1, NB):
            p1_body(i)

    cp_wo.wait()
    cp_win.wait()
    cp_b.wait()
    ri = lax.broadcasted_iota(jnp.int32, (G, G), 0) // DH
    ci = lax.broadcasted_iota(jnp.int32, (G, G), 1) // DH
    mask = ri == ci
    if NDEF >= 1:
        qproj(NB - 1)
    zcol = jnp.sum(zs_v[...], axis=-1, keepdims=True)
    for j in range(NG):
        zj = jnp.broadcast_to(zcol[j * G:(j + 1) * G, :], (G, G))
        zm_v[j * G:(j + 1) * G, :] = jnp.where(mask, zj, 0.0).astype(bf16)
    for j in range(NG):
        kvj = jnp.where(mask, kv_v[j * G:(j + 1) * G, :], 0.0).astype(bf16)
        m_v[j * G:(j + 1) * G, :] = _dot(kvj, wo_v[j * G:(j + 1) * G, :]).astype(bf16)

    NC = 4
    CH = S // NC

    def chain(i, fill=None):
        def gupd(c):
            if fill is None:
                k = NB - 2 - c
                if c < 2 and k >= NB - NDEF:
                    qproj(k)
                return
            rk = rows(fill)
            rc = slice(c * CH, (c + 1) * CH)
            g_v[rc, :] = jnp.where(fill == 0, 0.0, g_v[rc, :]) + _dot(wsp_v[rc, rk], z2_v[rk, :])

        r = rows(i)
        pq = pq_v[r, :]
        dens = [_dot(pq[:, j * G:(j + 1) * G], zm_v[j * G:(j + 1) * G, :]) for j in range(NG)]
        gupd(0)
        den = jnp.concatenate(dens, axis=-1) + 1e-6
        a = _div(pq.astype(f32), den).astype(bf16)
        h = x_v[r, :].astype(f32) + _dot(a, m_v[...])
        gupd(1)
        h_v[r, :] = h
        hn = _ln(h).astype(bf16)
        t2 = _dot(hn, win_v[:, FH:F])
        gupd(2)
        z2_v[r, :] = _ln(_gelu(t2)).astype(bf16)
        t1 = _dot(hn, win_v[:, 0:FH])
        gupd(3)
        z1_v[r, :] = _gelu(t1).astype(bf16)

    with _scope('P2a'):
        chain(0)
    cp_sp.wait()

    def p2(i, c):
        chain(i, i - 1)
        return c

    with _scope('P2'):
        lax.fori_loop(1, NB, p2, 0)

    cp_wout.wait()

    b = b_v[...].astype(f32)
    kl = slice((NB - 1) * TM, NB * TM)
    with _scope('P3'):
        for i in range(NB):
            r = rows(i)
            bcs = [jnp.broadcast_to(b[t:t + 1, :], (128, 128)).T for t in range(i * TM // 128, (i + 1) * TM // 128)]
            bc = jnp.concatenate(bcs, axis=0)
            g = g_v[r, :] + _dot(wsp_v[r, kl], z2_v[kl, :]) + jnp.concatenate([bc] * (FH // 128), axis=-1)
            y = (z1_v[r, :].astype(f32) * g).astype(bf16)
            out_v[r, :] = (h_v[r, :] + _dot(y, wout_v[...])).astype(bf16)
            cp_o(i).start()
    for i in range(NB):
        cp_o(i).wait()


@jax.jit
def pallas_sequential_preLN__linear_attn_block__mixer_gmlp__prompt_kernel(
    A_x, A_wqkv, A_wo, B_x, B_w_in, B_w_sp, B_b_sp, B_w_out,
):
    del B_x
    x = A_x.reshape(S, D)
    b = B_b_sp.reshape(S // 128, 128)
    any_spec = pl.BlockSpec(memory_space=pl.ANY)
    out = pl.pallas_call(
        _kernel,
        out_shape=jax.ShapeDtypeStruct((S, D), bf16),
        in_specs=[any_spec] * 7,
        out_specs=any_spec,
        scratch_shapes=[
            pltpu.VMEM((S, D), bf16),
            pltpu.VMEM((D, 3 * D), bf16),
            pltpu.VMEM((D, D), bf16),
            pltpu.VMEM((D, F), bf16),
            pltpu.VMEM((S, S), bf16),
            pltpu.VMEM((S // 128, 128), bf16),
            pltpu.VMEM((FH, D), bf16),
            pltpu.VMEM((D, D), bf16),
            pltpu.VMEM((S, D), bf16),
            pltpu.VMEM((D, S), bf16),
            pltpu.VMEM((S, D), bf16),
            pltpu.VMEM((D, G), f32),
            pltpu.VMEM((D, 128), f32),
            pltpu.VMEM((D, D), bf16),
            pltpu.VMEM((D, G), bf16),
            pltpu.VMEM((S, D), f32),
            pltpu.VMEM((S, FH), bf16),
            pltpu.VMEM((S, FH), bf16),
            pltpu.VMEM((S, FH), f32),
            pltpu.VMEM((S, D), bf16),
            pltpu.SemaphoreType.DMA((11,)),
            pltpu.SemaphoreType.DMA((NB,)),
        ],
        compiler_params=pltpu.CompilerParams(vmem_limit_bytes=100 * 1024 * 1024),
    )(x, A_wqkv, A_wo, B_w_in, B_w_sp, b, B_w_out)
    return out.reshape(1, S, D)
```

```python
import jax
import jax.numpy as jnp
from jax import lax
import jax.experimental.pallas as pl
import jax.experimental.pallas.tpu as pltpu

S, D, H, DH = 2048, 512, 32, 16
F, FH = 1792, 896
TM = 256
NB = S // TM
G = 128
NG = D // G
HD = D // 2
NDEF = 3
UC = 128
NC = 4
CH = S // NC
NS = 4
CW = D // NS

f32 = jnp.float32
bf16 = jnp.bfloat16


def _ln(x):
    m = jnp.mean(x, axis=-1, keepdims=True)
    xc = x - m
    v = jnp.mean(xc * xc, axis=-1, keepdims=True)
    return xc * lax.rsqrt(v + 1e-5)


def _phi(t):
    return jnp.where(t > 0, t + 1.0, jnp.exp(t)) + 1e-6


def _gelu(x):
    c = 0.7978845608028654
    return 0.5 * x * (1.0 + jnp.tanh(c * (x + 0.044715 * (x * x * x))))


def _dot(a, b):
    return jnp.dot(a, b, preferred_element_type=f32)


def _dot_nt(a, b):
    return lax.dot_general(a, b, (((1,), (1,)), ((), ())), preferred_element_type=f32)


def _div(a, b):
    r = pl.reciprocal(b, approx=True)
    r = r * (2.0 - b * r)
    return a * r


def _kernel(x_hbm, wqkv_hbm, wo_hbm, win_hbm, wsp_hbm, b_hbm, wout_hbm, out_hbm,
            x_v, wqkv_v, wo_v, win_v, wsp_v, b_v, wout_v,
            wkT_v, xn_v, pkT_v, pq_v, a_v, zs_v, m_v, zm_v, u_v, h_v, z1_v, z2_v, g_v, out_v,
            sem, sem_o):
    def rows(i):
        if isinstance(i, int):
            return pl.ds(i * TM, TM)
        return pl.ds(pl.multiple_of(i * TM, TM), TM)

    def cp_xr(lo, n, s):
        r = pl.ds(lo * TM, n * TM)
        return pltpu.make_async_copy(x_hbm.at[r], x_v.at[r], sem.at[s])

    def cp_wcols(lo, n, s):
        c = pl.ds(lo, n)
        return pltpu.make_async_copy(wqkv_hbm.at[:, c], wqkv_v.at[:, c], sem.at[s])

    def cp_o(i):
        r = pl.ds(i * TM, TM)
        return pltpu.make_async_copy(out_v.at[r], out_hbm.at[r], sem_o.at[i])

    def cp_ol(t):
        r = pl.ds((NB - 1) * TM, TM)
        c = pl.ds(t * CW, CW)
        return pltpu.make_async_copy(out_v.at[r, c], out_hbm.at[r, c], sem_o.at[NB - 1 + t])

    cp_x0 = cp_xr(0, 1, 0)
    cp_x1 = cp_xr(1, 1, 1)
    cp_x2 = cp_xr(2, NB - 2, 2)
    cp_wqa = cp_wcols(0, HD, 3)
    cp_wqb = cp_wcols(HD, HD, 4)
    cp_wk = cp_wcols(D, D, 5)
    cp_wv = cp_wcols(2 * D, D, 6)
    cp_wo = pltpu.make_async_copy(wo_hbm, wo_v, sem.at[7])
    cp_win = pltpu.make_async_copy(win_hbm, win_v, sem.at[8])
    cp_wout = pltpu.make_async_copy(wout_hbm, wout_v, sem.at[9])
    cp_b = pltpu.make_async_copy(b_hbm, b_v, sem.at[10])
    cp_sp = pltpu.make_async_copy(wsp_hbm, wsp_v, sem.at[11])

    cp_x0.start()
    cp_wqa.start()
    cp_wqb.start()
    cp_x1.start()
    cp_wk.start()
    cp_x2.start()

    def lnx(i):
        r = rows(i)
        xn_v[r, :] = _ln(x_v[r, :].astype(f32)).astype(bf16)

    def kproj(i):
        r = rows(i)
        pkT = _phi(_dot_nt(wkT_v[...], xn_v[r, :]))
        zpart = pkT[:, 0:128]
        for t in range(1, TM // 128):
            zpart = zpart + pkT[:, t * 128:(t + 1) * 128]
        if i == 0:
            zs_v[...] = zpart
        else:
            zs_v[...] += zpart
        pkT_v[:, r] = pkT.astype(bf16)

    def qproj(i, lo=0, hi=D):
        r = rows(i)
        pq_v[r, lo:hi] = _phi(_dot(xn_v[r, :], wqkv_v[:, lo:hi])).astype(bf16)

    def aupd(i):
        r2 = pl.ds(i * TM, 2 * TM)
        t = _dot(pkT_v[:, r2], xn_v[r2, :])
        if i == 0:
            a_v[...] = t
        else:
            a_v[...] += t

    cp_x0.wait()
    lnx(0)
    cp_wqa.wait()
    qproj(0, 0, HD)
    cp_wqb.wait()
    cp_x1.wait()
    qproj(0, HD, D)
    lnx(1)
    qproj(1, 0, HD)
    cp_wk.wait()
    qproj(1, HD, D)
    wkT_v[...] = wqkv_v[:, D:2 * D].astype(f32).T.astype(bf16)
    kproj(0)
    kproj(1)
    cp_x2.wait()
    cp_wv.start()
    cp_wo.start()
    cp_win.start()
    cp_b.start()
    cp_sp.start(priority=1)
    cp_wout.start(priority=1)

    for i in range(2, NB, 2):
        aupd(i - 2)
        for c in (i, i + 1):
            lnx(c)
            if c < NB - NDEF:
                qproj(c)
            kproj(c)
    aupd(NB - 2)

    cp_wv.wait()
    cp_wo.wait()
    cp_win.wait()
    cp_b.wait()
    ri = lax.broadcasted_iota(jnp.int32, (G, G), 0) // DH
    ci = lax.broadcasted_iota(jnp.int32, (G, G), 1) // DH
    mask = ri == ci
    kvs = [_dot(a_v[j * G:(j + 1) * G, :].astype(bf16), wqkv_v[:, 2 * D + j * G:2 * D + (j + 1) * G])
           for j in range(NG)]
    qproj(NB - 1)
    zcol = jnp.sum(zs_v[...], axis=-1, keepdims=True)
    for j in range(NG):
        zj = jnp.broadcast_to(zcol[j * G:(j + 1) * G, :], (G, G))
        zm_v[j * G:(j + 1) * G, :] = jnp.where(mask, zj, 0.0).astype(bf16)
    for j in range(NG):
        kvj = jnp.where(mask, kvs[j], 0.0).astype(bf16)
        m_v[j * G:(j + 1) * G, :] = _dot(kvj, wo_v[j * G:(j + 1) * G, :]).astype(bf16)

    def chain(i, prev=None):
        def filler(c):
            if prev is None:
                if c < NDEF - 1:
                    qproj(NB - 2 - c)
                return
            rk = rows(prev)
            rc = slice(c * CH, (c + 1) * CH)
            g_v[rc, :] = jnp.where(prev == 0, 0.0, g_v[rc, :]) + _dot(wsp_v[rc, rk], z2_v[rk, :])

        r = rows(i)
        pq = pq_v[r, :]
        dens = [_dot(pq[:, j * G:(j + 1) * G], zm_v[j * G:(j + 1) * G, :]) for j in range(NG)]
        filler(0)
        den = jnp.concatenate(dens, axis=-1) + 1e-6
        a = _div(pq.astype(f32), den).astype(bf16)
        h = x_v[r, :].astype(f32) + _dot(a, m_v[...])
        filler(1)
        h_v[r, :] = h
        hn = _ln(h).astype(bf16)
        for c in range(FH // UC):
            u_v[:, c * UC:(c + 1) * UC] = _gelu(_dot(hn, win_v[:, FH + c * UC:FH + (c + 1) * UC]))
        filler(2)
        m2 = jnp.mean(u_v[...], axis=-1, keepdims=True)
        uc = u_v[...] - m2
        rs = lax.rsqrt(jnp.mean(uc * uc, axis=-1, keepdims=True) + 1e-5)
        z2_v[r, :] = (u_v[...] * rs - m2 * rs).astype(bf16)
        t1 = _dot(hn, win_v[:, 0:FH])
        filler(3)
        z1_v[r, :] = _gelu(t1).astype(bf16)

    chain(0)
    cp_sp.wait()

    def p2(i, c):
        chain(i, i - 1)
        return c

    lax.fori_loop(1, NB, p2, 0)

    cp_wout.wait()

    b = b_v[...].astype(f32)
    kl = slice((NB - 1) * TM, NB * TM)
    for i in range(NB):
        r = rows(i)
        bcs = [jnp.broadcast_to(b[t:t + 1, :], (128, 128)).T
               for t in range(i * TM // 128, (i + 1) * TM // 128)]
        bc = jnp.concatenate(bcs, axis=0)
        g = g_v[r, :] + _dot(wsp_v[r, kl], z2_v[kl, :]) + jnp.concatenate([bc] * (FH // 128), axis=-1)
        y = (z1_v[r, :].astype(f32) * g).astype(bf16)
        if i < NB - 1:
            out_v[r, :] = (h_v[r, :] + _dot(y, wout_v[...])).astype(bf16)
            cp_o(i).start()
        else:
            for t in range(NS):
                cs = slice(t * CW, (t + 1) * CW)
                out_v[r, cs] = (h_v[r, cs] + _dot(y, wout_v[:, cs])).astype(bf16)
                cp_ol(t).start()
    for i in range(NB - 1):
        cp_o(i).wait()
    for t in range(NS):
        cp_ol(t).wait()


@jax.jit
def pallas_sequential_preLN__linear_attn_block__mixer_gmlp__prompt_kernel(
    A_x: jax.Array,
    A_wqkv: jax.Array,
    A_wo: jax.Array,
    B_x: jax.Array,
    B_w_in: jax.Array,
    B_w_sp: jax.Array,
    B_b_sp: jax.Array,
    B_w_out: jax.Array,
):
    del B_x
    x = A_x.reshape(S, D)
    b = B_b_sp.reshape(S // 128, 128)
    any_spec = pl.BlockSpec(memory_space=pl.ANY)
    out = pl.pallas_call(
        _kernel,
        out_shape=jax.ShapeDtypeStruct((S, D), bf16),
        in_specs=[any_spec] * 7,
        out_specs=any_spec,
        scratch_shapes=[
            pltpu.VMEM((S, D), bf16),
            pltpu.VMEM((D, 3 * D), bf16),
            pltpu.VMEM((D, D), bf16),
            pltpu.VMEM((D, F), bf16),
            pltpu.VMEM((S, S), bf16),
            pltpu.VMEM((S // 128, 128), bf16),
            pltpu.VMEM((FH, D), bf16),
            pltpu.VMEM((D, D), bf16),
            pltpu.VMEM((S, D), bf16),
            pltpu.VMEM((D, S), bf16),
            pltpu.VMEM((S, D), bf16),
            pltpu.VMEM((D, D), f32),
            pltpu.VMEM((D, 128), f32),
            pltpu.VMEM((D, D), bf16),
            pltpu.VMEM((D, G), bf16),
            pltpu.VMEM((TM, FH), f32),
            pltpu.VMEM((S, D), f32),
            pltpu.VMEM((S, FH), bf16),
            pltpu.VMEM((S, FH), bf16),
            pltpu.VMEM((S, FH), f32),
            pltpu.VMEM((S, D), bf16),
            pltpu.SemaphoreType.DMA((12,)),
            pltpu.SemaphoreType.DMA((NB - 1 + NS,)),
        ],
        compiler_params=pltpu.CompilerParams(vmem_limit_bytes=100 * 1024 * 1024),
    )(x, A_wqkv, A_wo, B_w_in, B_w_sp, b, B_w_out)
    return out.reshape(1, S, D)
```
